```python
import os as _os
_os.environ.setdefault("JAX_PLATFORMS", "cpu")
import jax
import jax.numpy as jnp

def _softmax(x, axis=-1):
    return jax.nn.softmax(x, axis=axis)
def _gelu(x):
    return jax.nn.gelu(x, approximate=True)
def _silu(x):
    return jax.nn.silu(x)
def _sigmoid(x):
    return jax.nn.sigmoid(x)
def _layernorm(x, axis=-1, eps=1e-5):
    m = jnp.mean(x, axis=axis, keepdims=True)
    v = jnp.var(x, axis=axis, keepdims=True)
    return (x - m) / jnp.sqrt(v + eps)
def _scatter_add(tgt, idx, src, axis=0):
    return tgt.at[idx].add(src)
def _segment_sum(src, seg, n):
    return jax.ops.segment_sum(src, seg, n)
class _Rng:
    def __init__(self, key):
        self._k = key
    def _next(self):
        self._k, sub = jax.random.split(self._k)
        return sub
    def normal(self, shape):
        return jax.random.normal(self._next(), shape, dtype=jnp.bfloat16)
    def randint(self, lo, hi, shape):
        return jax.random.randint(self._next(), shape, lo, hi, dtype=jnp.int32)
    def uniform(self, shape, lo=0.0, hi=1.0):
        return jax.random.uniform(self._next(), shape, jnp.bfloat16, lo, hi)
    def permutation(self, n):
        return jax.random.permutation(self._next(), n)


kernel_name = 'concat_heads__gqa_block_cached__gqa_block_cached__near_ridge'

def setup_inputs():
    _rng = _Rng(jax.random.key(int.from_bytes(__import__("os").urandom(4), "little")))
    _w = (lambda a: (lambda t: t.astype(jnp.bfloat16) if jnp.issubdtype(t.dtype, jnp.floating) else t)(jnp.asarray(a)))
    def _A_setup():
        B, Sq, D = 8, 240, 640
        Hq, Hkv, Sk, Dh = 32, 32, 1024, 192
        assert Hq % Hkv == 0, (Hq, Hkv)
        return {
            "x": _w((lambda *s: _rng.normal(s) * 0.8)(B, Sq, D)),
            "k_cache": _w((lambda *s: _rng.normal(s) * 0.8)(B, Hkv, Sk, Dh)),
            "v_cache": _w((lambda *s: _rng.normal(s) * 0.05)(B, Hkv, Sk, Dh)),
            "wq": _w((lambda *s: _rng.normal(s) * 0.8)(D, Hq * Dh) * (D ** -0.5)),
            "wo": _w((lambda *s: _rng.normal(s) * 0.05)(Hq * Dh, D) * ((Hq * Dh) ** -0.5)),
        }
    _A_in = _A_setup()

    def _B_setup():
        B, Sq, D = 8, 240, 640
        Hq, Hkv, Sk, Dh = 32, 32, 1024, 192
        assert Hq % Hkv == 0, (Hq, Hkv)
        return {
            "x": _w((lambda *s: _rng.normal(s) * 0.8)(B, Sq, D)),
            "k_cache": _w((lambda *s: _rng.normal(s) * 0.8)(B, Hkv, Sk, Dh)),
            "v_cache": _w((lambda *s: _rng.normal(s) * 0.05)(B, Hkv, Sk, Dh)),
            "wq": _w((lambda *s: _rng.normal(s) * 0.8)(D, Hq * Dh) * (D ** -0.5)),
            "wo": _w((lambda *s: _rng.normal(s) * 0.05)(Hq * Dh, D) * ((Hq * Dh) ** -0.5)),
        }
    _B_in = _B_setup()

    return {
        "A_x": _A_in["x"],
        "A_k_cache": _A_in["k_cache"],
        "A_v_cache": _A_in["v_cache"],
        "A_wq": _A_in["wq"],
        "A_wo": _A_in["wo"],
        "B_x": _B_in["x"],
        "B_k_cache": _B_in["k_cache"],
        "B_v_cache": _B_in["v_cache"],
        "B_wq": _B_in["wq"],
        "B_wo": _B_in["wo"],
    }

def reference(A_x, A_k_cache, A_v_cache, A_wq, A_wo, B_x, B_k_cache, B_v_cache, B_wq, B_wo):
    def _A_ref(x, k_cache, v_cache, wq, wo):
        B, Sq, D = x.shape
        Hq, Dh = 32, 192
        Hkv = k_cache.shape[1]
        rep = Hq // Hkv
        q = (lambda x, *d: x.transpose(*d))((x @ wq).reshape(B, Sq, Hq, Dh), 0, 2, 1, 3)
        k = jnp.repeat(k_cache, rep, axis=1)
        v = jnp.repeat(v_cache, rep, axis=1)
        scores = jnp.einsum("bhqd,bhkd->bhqk", q, k) * (Dh ** -0.5)
        p = _softmax(scores, axis=-1)
        o = jnp.einsum("bhqk,bhkd->bhqd", p, v)
        return (lambda x, *d: x.transpose(*d))(o, 0, 2, 1, 3).reshape(B, Sq, Hq * Dh) @ wo

    def _B_ref(x, k_cache, v_cache, wq, wo):
        B, Sq, D = x.shape
        Hq, Dh = 32, 192
        Hkv = k_cache.shape[1]
        rep = Hq // Hkv
        q = (lambda x, *d: x.transpose(*d))((x @ wq).reshape(B, Sq, Hq, Dh), 0, 2, 1, 3)
        k = jnp.repeat(k_cache, rep, axis=1)
        v = jnp.repeat(v_cache, rep, axis=1)
        scores = jnp.einsum("bhqd,bhkd->bhqk", q, k) * (Dh ** -0.5)
        p = _softmax(scores, axis=-1)
        o = jnp.einsum("bhqk,bhkd->bhqd", p, v)
        return (lambda x, *d: x.transpose(*d))(o, 0, 2, 1, 3).reshape(B, Sq, Hq * Dh) @ wo

    a = _A_ref(A_x, A_k_cache, A_v_cache, A_wq, A_wo)
    b = _B_ref(B_x, B_k_cache, B_v_cache, B_wq, B_wo)
    return jnp.concatenate([a, b], axis=-1)
```

```python
import functools

import jax
import jax.numpy as jnp
import jax.experimental.pallas as pl
import jax.experimental.pallas.tpu as pltpu

HQ = 32
DH = 192
HP = 2


def _attn_kernel(xa_ref, ka_ref, va_ref, wqa_ref, woa_ref,
                 xb_ref, kb_ref, vb_ref, wqb_ref, wob_ref,
                 o_ref, acca_ref, accb_ref, *, d_model):
    hp = pl.program_id(1)
    n_hp = pl.num_programs(1)
    scale = DH ** -0.5
    w = HP * DH

    def one(x_ref, k_ref, v_ref, wq_ref, wo_ref, acc_ref):
        x = x_ref[0]
        col = pl.multiple_of(hp * w, 128)
        q2 = jnp.dot(x, wq_ref[:, pl.ds(col, w)], preferred_element_type=jnp.float32)
        q2 = (q2 * scale).astype(jnp.bfloat16)
        outs = []
        for j in range(HP):
            q = q2[:, j * DH:(j + 1) * DH]
            k = k_ref[0, j]
            v = v_ref[0, j]
            s = jax.lax.dot_general(q, k, (((1,), (1,)), ((), ())),
                                    preferred_element_type=jnp.float32)
            m = jnp.max(s, axis=-1, keepdims=True)
            p = jnp.exp(s - m)
            l = jnp.sum(p, axis=-1, keepdims=True)
            o = jnp.dot(p.astype(jnp.bfloat16), v, preferred_element_type=jnp.float32)
            outs.append((o / l).astype(jnp.bfloat16))
        o2 = jnp.concatenate(outs, axis=-1)
        contrib = jnp.dot(o2, wo_ref[pl.ds(col, w), :], preferred_element_type=jnp.float32)

        @pl.when(hp == 0)
        def _():
            acc_ref[...] = contrib

        @pl.when(hp != 0)
        def _():
            acc_ref[...] += contrib

    one(xa_ref, ka_ref, va_ref, wqa_ref, woa_ref, acca_ref)
    one(xb_ref, kb_ref, vb_ref, wqb_ref, wob_ref, accb_ref)

    @pl.when(hp == n_hp - 1)
    def _():
        o_ref[0, :, :d_model] = acca_ref[...].astype(o_ref.dtype)
        o_ref[0, :, d_model:] = accb_ref[...].astype(o_ref.dtype)


@jax.jit
def pallas_concat_heads__gqa_block_cached__gqa_block_cached__near_ridge_kernel(
    A_x: jax.Array,
    A_k_cache: jax.Array,
    A_v_cache: jax.Array,
    A_wq: jax.Array,
    A_wo: jax.Array,
    B_x: jax.Array,
    B_k_cache: jax.Array,
    B_v_cache: jax.Array,
    B_wq: jax.Array,
    B_wo: jax.Array,
):
    B, Sq, D = A_x.shape
    _, Hkv, Sk, Dh = A_k_cache.shape
    assert Hkv == HQ and Dh == DH

    x_spec = pl.BlockSpec((1, Sq, D), lambda b, h: (b, 0, 0))
    kv_spec = pl.BlockSpec((1, HP, Sk, Dh), lambda b, h: (b, h, 0, 0))
    wq_spec = pl.BlockSpec((D, HQ * DH), lambda b, h: (0, 0))
    wo_spec = pl.BlockSpec((HQ * DH, D), lambda b, h: (0, 0))
    in_specs = [x_spec, kv_spec, kv_spec, wq_spec, wo_spec] * 2

    return pl.pallas_call(
        functools.partial(_attn_kernel, d_model=D),
        grid=(B, HQ // HP),
        in_specs=in_specs,
        out_specs=pl.BlockSpec((1, Sq, 2 * D), lambda b, h: (b, 0, 0)),
        out_shape=jax.ShapeDtypeStruct((B, Sq, 2 * D), A_x.dtype),
        scratch_shapes=[
            pltpu.VMEM((Sq, D), jnp.float32),
            pltpu.VMEM((Sq, D), jnp.float32),
        ],
        compiler_params=pltpu.CompilerParams(
            dimension_semantics=("arbitrary", "arbitrary"),
            vmem_limit_bytes=100 * 1024 * 1024,
        ),
    )(A_x, A_k_cache, A_v_cache, A_wq, A_wo,
      B_x, B_k_cache, B_v_cache, B_wq, B_wo)
```

```python
import functools

import jax
import jax.numpy as jnp
import jax.experimental.pallas as pl
import jax.experimental.pallas.tpu as pltpu

HQ = 32
DH = 192
HP = 2


def _attn_kernel(xa_ref, ka_ref, va_ref, wqa_ref, woa_ref,
                 xb_ref, kb_ref, vb_ref, wqb_ref, wob_ref,
                 o_ref, acca_ref, accb_ref, *, d_model):
    hp = pl.program_id(1)
    n_hp = pl.num_programs(1)
    scale = DH ** -0.5
    w = HP * DH

    def one(x_ref, kt_ref, vt_ref, wq_ref, wo_ref, acc_ref):
        x = x_ref[0]
        col = pl.multiple_of(hp * w, 128)
        q2 = jnp.dot(x, wq_ref[:, pl.ds(col, w)], preferred_element_type=jnp.float32)
        q2 = (q2 * scale).astype(jnp.bfloat16)
        outs = []
        for j in range(HP):
            q = q2[:, j * DH:(j + 1) * DH]
            kt = kt_ref[0, j]
            vt = vt_ref[0, j]
            s = jnp.dot(q, kt, preferred_element_type=jnp.float32)
            m = jnp.max(s, axis=-1, keepdims=True)
            p = jnp.exp(s - m)
            l = jnp.sum(p, axis=-1, keepdims=True)
            o = jax.lax.dot_general(p.astype(jnp.bfloat16), vt, (((1,), (1,)), ((), ())),
                                    preferred_element_type=jnp.float32)
            outs.append((o / l).astype(jnp.bfloat16))
        o2 = jnp.concatenate(outs, axis=-1)
        contrib = jnp.dot(o2, wo_ref[pl.ds(col, w), :], preferred_element_type=jnp.float32)

        @pl.when(hp == 0)
        def _():
            acc_ref[...] = contrib

        @pl.when(hp != 0)
        def _():
            acc_ref[...] += contrib

    one(xa_ref, ka_ref, va_ref, wqa_ref, woa_ref, acca_ref)
    one(xb_ref, kb_ref, vb_ref, wqb_ref, wob_ref, accb_ref)

    @pl.when(hp == n_hp - 1)
    def _():
        o_ref[0, :, :d_model] = acca_ref[...].astype(o_ref.dtype)
        o_ref[0, :, d_model:] = accb_ref[...].astype(o_ref.dtype)


@jax.jit
def pallas_concat_heads__gqa_block_cached__gqa_block_cached__near_ridge_kernel(
    A_x: jax.Array,
    A_k_cache: jax.Array,
    A_v_cache: jax.Array,
    A_wq: jax.Array,
    A_wo: jax.Array,
    B_x: jax.Array,
    B_k_cache: jax.Array,
    B_v_cache: jax.Array,
    B_wq: jax.Array,
    B_wo: jax.Array,
):
    B, Sq, D = A_x.shape
    _, Hkv, Sk, Dh = A_k_cache.shape
    assert Hkv == HQ and Dh == DH

    kta = jnp.swapaxes(A_k_cache, 2, 3)
    vta = jnp.swapaxes(A_v_cache, 2, 3)
    ktb = jnp.swapaxes(B_k_cache, 2, 3)
    vtb = jnp.swapaxes(B_v_cache, 2, 3)

    x_spec = pl.BlockSpec((1, Sq, D), lambda b, h: (b, 0, 0))
    kv_spec = pl.BlockSpec((1, HP, Dh, Sk), lambda b, h: (b, h, 0, 0))
    wq_spec = pl.BlockSpec((D, HQ * DH), lambda b, h: (0, 0))
    wo_spec = pl.BlockSpec((HQ * DH, D), lambda b, h: (0, 0))
    in_specs = [x_spec, kv_spec, kv_spec, wq_spec, wo_spec] * 2

    return pl.pallas_call(
        functools.partial(_attn_kernel, d_model=D),
        grid=(B, HQ // HP),
        in_specs=in_specs,
        out_specs=pl.BlockSpec((1, Sq, 2 * D), lambda b, h: (b, 0, 0)),
        out_shape=jax.ShapeDtypeStruct((B, Sq, 2 * D), A_x.dtype),
        scratch_shapes=[
            pltpu.VMEM((Sq, D), jnp.float32),
            pltpu.VMEM((Sq, D), jnp.float32),
        ],
        compiler_params=pltpu.CompilerParams(
            dimension_semantics=("arbitrary", "arbitrary"),
            vmem_limit_bytes=100 * 1024 * 1024,
        ),
    )(A_x, kta, vta, A_wq, A_wo,
      B_x, ktb, vtb, B_wq, B_wo)
```

```python
import functools

import jax
import jax.numpy as jnp
import jax.experimental.pallas as pl
import jax.experimental.pallas.tpu as pltpu

HQ = 32
DH = 192
HP = 2
NHP = HQ // HP
ROWS = 48


def _attn_kernel(xa_ref, kta_ref, vta_ref, wqa_ref, woa_ref,
                 xb_ref, ktb_ref, vtb_ref, wqb_ref, wob_ref,
                 o_ref, s0_ref, s1_ref, p0_ref, p1_ref, acca_ref, accb_ref,
                 *, d_model, n_steps):
    t = pl.program_id(0)
    scale = DH ** -0.5
    w = HP * DH
    sq = xa_ref.shape[1]
    hp_q = jnp.minimum(t, n_steps - 1) % NHP
    hp_p = jnp.maximum(t - 2, 0) % NHP

    @pl.when(t == 0)
    def _():
        for r in (s0_ref, s1_ref, p0_ref, p1_ref):
            r[...] = jnp.zeros(r.shape, r.dtype)

    probs = ((xa_ref, kta_ref, vta_ref, wqa_ref, woa_ref, acca_ref),
             (xb_ref, ktb_ref, vtb_ref, wqb_ref, wob_ref, accb_ref))

    def step(s_wr, s_rd, p_wr, p_rd):
        colq = pl.multiple_of(hp_q * w, 128)
        colp = pl.multiple_of(hp_p * w, 128)
        nt = s_wr.shape[-1] // 128
        z = 0
        for pi, (x_ref, kt_ref, vt_ref, wq_ref, wo_ref, acc_ref) in enumerate(probs):
            q2 = jnp.dot(x_ref[0], wq_ref[:, pl.ds(colq, w)],
                         preferred_element_type=jnp.float32)
            q2 = (q2 * scale).astype(jnp.bfloat16)
            outs = []
            for j in range(HP):
                i = pi * HP + j
                q = q2[:, j * DH:(j + 1) * DH]
                o = None
                for c in range(nt):
                    cs = slice(c * 128, (c + 1) * 128)
                    s_wr[i, :, cs] = jnp.dot(q, kt_ref[0, j + z, :, cs],
                                             preferred_element_type=jnp.float32)
                    oc = jax.lax.dot_general(p_rd[i, :, cs], vt_ref[0, j, :, cs],
                                             (((1,), (1,)), ((), ())),
                                             preferred_element_type=jnp.float32)
                    o = oc if o is None else o + oc
                    r0 = c * ROWS
                    if r0 < sq:
                        s = s_rd[i, r0:r0 + ROWS, :]
                        m = jnp.max(s, axis=-1, keepdims=True)
                        e = jnp.exp(s - m)
                        l = jnp.sum(e, axis=-1, keepdims=True)
                        p_wr[i, r0:r0 + ROWS, :] = (e * (1.0 / l)).astype(jnp.bfloat16)
                        z = (jnp.min(l) < 0.0).astype(jnp.int32)
                outs.append(o.astype(jnp.bfloat16))
            o2 = jnp.concatenate(outs, axis=-1)
            contrib = jnp.dot(o2, wo_ref[pl.ds(colp, w), :],
                              preferred_element_type=jnp.float32)
            acc_ref[...] = jnp.where(hp_p == 0, 0.0, acc_ref[...]) + contrib

    @pl.when(t % 2 == 0)
    def _():
        step(s0_ref, s1_ref, p1_ref, p0_ref)

    @pl.when(t % 2 == 1)
    def _():
        step(s1_ref, s0_ref, p0_ref, p1_ref)

    @pl.when(jnp.logical_and(t >= 2, hp_p == NHP - 1))
    def _():
        o_ref[0, :, :d_model] = acca_ref[...].astype(o_ref.dtype)
        o_ref[0, :, d_model:] = accb_ref[...].astype(o_ref.dtype)


@jax.jit
def pallas_concat_heads__gqa_block_cached__gqa_block_cached__near_ridge_kernel(
    A_x: jax.Array,
    A_k_cache: jax.Array,
    A_v_cache: jax.Array,
    A_wq: jax.Array,
    A_wo: jax.Array,
    B_x: jax.Array,
    B_k_cache: jax.Array,
    B_v_cache: jax.Array,
    B_wq: jax.Array,
    B_wo: jax.Array,
):
    B, Sq, D = A_x.shape
    _, Hkv, Sk, Dh = A_k_cache.shape
    assert Hkv == HQ and Dh == DH
    n_steps = B * NHP

    kta = jnp.swapaxes(A_k_cache, 2, 3)
    vta = jnp.swapaxes(A_v_cache, 2, 3)
    ktb = jnp.swapaxes(B_k_cache, 2, 3)
    vtb = jnp.swapaxes(B_v_cache, 2, 3)

    def tq(t):
        return jnp.minimum(t, n_steps - 1)

    def tp(t):
        return jnp.maximum(t - 2, 0)

    x_spec = pl.BlockSpec((1, Sq, D), lambda t: (tq(t) // NHP, 0, 0))
    k_spec = pl.BlockSpec((1, HP, Dh, Sk), lambda t: (tq(t) // NHP, tq(t) % NHP, 0, 0))
    v_spec = pl.BlockSpec((1, HP, Dh, Sk), lambda t: (tp(t) // NHP, tp(t) % NHP, 0, 0))
    wq_spec = pl.BlockSpec((D, HQ * DH), lambda t: (0, 0))
    wo_spec = pl.BlockSpec((HQ * DH, D), lambda t: (0, 0))
    in_specs = [x_spec, k_spec, v_spec, wq_spec, wo_spec] * 2

    return pl.pallas_call(
        functools.partial(_attn_kernel, d_model=D, n_steps=n_steps),
        grid=(n_steps + 2,),
        in_specs=in_specs,
        out_specs=pl.BlockSpec((1, Sq, 2 * D), lambda t: (tp(t) // NHP, 0, 0)),
        out_shape=jax.ShapeDtypeStruct((B, Sq, 2 * D), A_x.dtype),
        scratch_shapes=[
            pltpu.VMEM((2 * HP, Sq, Sk), jnp.float32),
            pltpu.VMEM((2 * HP, Sq, Sk), jnp.float32),
            pltpu.VMEM((2 * HP, Sq, Sk), jnp.bfloat16),
            pltpu.VMEM((2 * HP, Sq, Sk), jnp.bfloat16),
            pltpu.VMEM((Sq, D), jnp.float32),
            pltpu.VMEM((Sq, D), jnp.float32),
        ],
        compiler_params=pltpu.CompilerParams(
            dimension_semantics=("arbitrary",),
            vmem_limit_bytes=100 * 1024 * 1024,
        ),
    )(A_x, kta, vta, A_wq, A_wo,
      B_x, ktb, vtb, B_wq, B_wo)
```

```python
import functools

import jax
import jax.numpy as jnp
import jax.experimental.pallas as pl
import jax.experimental.pallas.tpu as pltpu

HQ = 32
DH = 192
HP = 2
NHP = HQ // HP
ROWS = 48


def _attn_kernel(xa_ref, kta_ref, vta_ref, wqa_ref, woa_ref,
                 xb_ref, ktb_ref, vtb_ref, wqb_ref, wob_ref,
                 o_ref, s_ref, p_ref, acca_ref, accb_ref,
                 *, d_model, n_steps):
    t = pl.program_id(0)
    scale = DH ** -0.5
    w = HP * DH
    sq = xa_ref.shape[1]
    hp_q = jnp.minimum(t, n_steps - 1) % NHP
    hp_p = jnp.maximum(t - 2, 0) % NHP

    @pl.when(t == 0)
    def _():
        for r in (s_ref, p_ref):
            r[...] = jnp.zeros(r.shape, r.dtype)

    probs = ((xa_ref, kta_ref, vta_ref, wqa_ref, woa_ref, acca_ref),
             (xb_ref, ktb_ref, vtb_ref, wqb_ref, wob_ref, accb_ref))

    def step(s_wr, s_rd, p_wr, p_rd):
        colq = pl.multiple_of(hp_q * w, 128)
        colp = pl.multiple_of(hp_p * w, 128)
        nt = s_wr.shape[-1] // 128
        z = 0
        for pi, (x_ref, kt_ref, vt_ref, wq_ref, wo_ref, acc_ref) in enumerate(probs):
            q2 = jnp.dot(x_ref[0], wq_ref[:, pl.ds(colq, w)],
                         preferred_element_type=jnp.float32)
            q2 = (q2 * scale).astype(jnp.bfloat16)
            outs = []
            for j in range(HP):
                i = pi * HP + j
                q = q2[:, j * DH:(j + 1) * DH]
                o = None
                for c in range(nt):
                    cs = slice(c * 128, (c + 1) * 128)
                    s_wr[i, :, cs] = jnp.dot(q, kt_ref[0, j + z, :, cs],
                                             preferred_element_type=jnp.float32)
                    oc = jax.lax.dot_general(p_rd[i, :, cs], vt_ref[0, j, :, cs],
                                             (((1,), (1,)), ((), ())),
                                             preferred_element_type=jnp.float32)
                    o = oc if o is None else o + oc
                    r0 = c * ROWS
                    if r0 < sq:
                        s = s_rd[i, r0:r0 + ROWS, :]
                        m = jnp.max(s, axis=-1, keepdims=True)
                        e = jnp.exp(s - m)
                        l = jnp.sum(e, axis=-1, keepdims=True)
                        p_wr[i, r0:r0 + ROWS, :] = (e * (1.0 / l)).astype(jnp.bfloat16)
                        z = (jnp.min(l) < 0.0).astype(jnp.int32)
                outs.append(o.astype(jnp.bfloat16))
            o2 = jnp.concatenate(outs, axis=-1)
            contrib = jnp.dot(o2, wo_ref[pl.ds(colp, w), :],
                              preferred_element_type=jnp.float32)
            acc_ref[...] = jnp.where(hp_p == 0, 0.0, acc_ref[...]) + contrib

    cur = t % 2
    step(s_ref.at[cur], s_ref.at[1 - cur], p_ref.at[1 - cur], p_ref.at[cur])

    @pl.when(jnp.logical_and(t >= 2, hp_p == NHP - 1))
    def _():
        o_ref[0, :, :d_model] = acca_ref[...].astype(o_ref.dtype)
        o_ref[0, :, d_model:] = accb_ref[...].astype(o_ref.dtype)


@jax.jit
def pallas_concat_heads__gqa_block_cached__gqa_block_cached__near_ridge_kernel(
    A_x: jax.Array,
    A_k_cache: jax.Array,
    A_v_cache: jax.Array,
    A_wq: jax.Array,
    A_wo: jax.Array,
    B_x: jax.Array,
    B_k_cache: jax.Array,
    B_v_cache: jax.Array,
    B_wq: jax.Array,
    B_wo: jax.Array,
):
    B, Sq, D = A_x.shape
    _, Hkv, Sk, Dh = A_k_cache.shape
    assert Hkv == HQ and Dh == DH
    n_steps = B * NHP

    kta = jnp.swapaxes(A_k_cache, 2, 3)
    vta = jnp.swapaxes(A_v_cache, 2, 3)
    ktb = jnp.swapaxes(B_k_cache, 2, 3)
    vtb = jnp.swapaxes(B_v_cache, 2, 3)

    def tq(t):
        return jnp.minimum(t, n_steps - 1)

    def tp(t):
        return jnp.maximum(t - 2, 0)

    x_spec = pl.BlockSpec((1, Sq, D), lambda t: (tq(t) // NHP, 0, 0))
    k_spec = pl.BlockSpec((1, HP, Dh, Sk), lambda t: (tq(t) // NHP, tq(t) % NHP, 0, 0))
    v_spec = pl.BlockSpec((1, HP, Dh, Sk), lambda t: (tp(t) // NHP, tp(t) % NHP, 0, 0))
    wq_spec = pl.BlockSpec((D, HQ * DH), lambda t: (0, 0))
    wo_spec = pl.BlockSpec((HQ * DH, D), lambda t: (0, 0))
    in_specs = [x_spec, k_spec, v_spec, wq_spec, wo_spec] * 2

    return pl.pallas_call(
        functools.partial(_attn_kernel, d_model=D, n_steps=n_steps),
        grid=(n_steps + 2,),
        in_specs=in_specs,
        out_specs=pl.BlockSpec((1, Sq, 2 * D), lambda t: (tp(t) // NHP, 0, 0)),
        out_shape=jax.ShapeDtypeStruct((B, Sq, 2 * D), A_x.dtype),
        scratch_shapes=[
            pltpu.VMEM((2, 2 * HP, Sq, Sk), jnp.float32),
            pltpu.VMEM((2, 2 * HP, Sq, Sk), jnp.bfloat16),
            pltpu.VMEM((Sq, D), jnp.float32),
            pltpu.VMEM((Sq, D), jnp.float32),
        ],
        compiler_params=pltpu.CompilerParams(
            dimension_semantics=("arbitrary",),
            vmem_limit_bytes=100 * 1024 * 1024,
        ),
    )(A_x, kta, vta, A_wq, A_wo,
      B_x, ktb, vtb, B_wq, B_wo)
```

```python
import functools

import jax
import jax.numpy as jnp
import jax.experimental.pallas as pl
import jax.experimental.pallas.tpu as pltpu

HQ = 32
DH = 192
HP = 2
NHP = HQ // HP
ROWS = 48


def _attn_kernel(xa_ref, kta_ref, vta_ref, wqa_ref, woa_ref,
                 xb_ref, ktb_ref, vtb_ref, wqb_ref, wob_ref,
                 o_ref, s0_ref, s1_ref, p0_ref, p1_ref, acca_ref, accb_ref,
                 *, d_model, n_steps):
    t = pl.program_id(0)
    scale = DH ** -0.5
    w = HP * DH
    sq = xa_ref.shape[1]
    hp_q = jnp.minimum(t, n_steps - 1) % NHP
    hp_p = jnp.maximum(t - 2, 0) % NHP

    @pl.when(t == 0)
    def _():
        for r in (s0_ref, s1_ref, p0_ref, p1_ref):
            r[...] = jnp.zeros(r.shape, r.dtype)

    probs = ((xa_ref, kta_ref, vta_ref, wqa_ref, woa_ref, acca_ref),
             (xb_ref, ktb_ref, vtb_ref, wqb_ref, wob_ref, accb_ref))

    def step(s_wr, s_rd, p_wr, p_rd):
        colq = pl.multiple_of(hp_q * w, 128)
        colp = pl.multiple_of(hp_p * w, 128)
        nt = s_wr.shape[-1] // 128
        z = 0
        for pi, (x_ref, kt_ref, vt_ref, wq_ref, wo_ref, acc_ref) in enumerate(probs):
            q2 = jnp.dot(x_ref[0], wq_ref[:, pl.ds(colq, w)],
                         preferred_element_type=jnp.float32)
            q2 = (q2 * scale).astype(jnp.bfloat16)
            outs = []
            for j in range(HP):
                i = pi * HP + j
                q = q2[:, j * DH:(j + 1) * DH]
                o = None
                for c in range(nt):
                    cs = slice(c * 128, (c + 1) * 128)
                    s_wr[i, :, cs] = jnp.dot(q, kt_ref[0, j + z, :, cs],
                                             preferred_element_type=jnp.float32)
                    oc = jax.lax.dot_general(p_rd[i, :, cs], vt_ref[0, j, :, cs],
                                             (((1,), (1,)), ((), ())),
                                             preferred_element_type=jnp.float32)
                    o = oc if o is None else o + oc
                    r0 = c * ROWS
                    if r0 < sq:
                        s = s_rd[i, r0:r0 + ROWS, :]
                        m = jnp.max(s, axis=-1, keepdims=True)
                        e = jnp.exp(s - m)
                        l = jnp.sum(e, axis=-1, keepdims=True)
                        p_wr[i, r0:r0 + ROWS, :] = (e * (1.0 / l)).astype(jnp.bfloat16)
                        lmin = jnp.min(l) if r0 == 0 else jnp.minimum(lmin, jnp.min(l))
                z = (lmin < 0.0).astype(jnp.int32)
                outs.append(o.astype(jnp.bfloat16))
            o2 = jnp.concatenate(outs, axis=-1)
            contrib = jnp.dot(o2, wo_ref[pl.ds(colp, w), :],
                              preferred_element_type=jnp.float32)
            acc_ref[...] = jnp.where(hp_p == 0, 0.0, acc_ref[...]) + contrib

    @pl.when(t % 2 == 0)
    def _():
        step(s0_ref, s1_ref, p1_ref, p0_ref)

    @pl.when(t % 2 == 1)
    def _():
        step(s1_ref, s0_ref, p0_ref, p1_ref)

    @pl.when(jnp.logical_and(t >= 2, hp_p == NHP - 1))
    def _():
        o_ref[0, :, :d_model] = acca_ref[...].astype(o_ref.dtype)
        o_ref[0, :, d_model:] = accb_ref[...].astype(o_ref.dtype)


@jax.jit
def pallas_concat_heads__gqa_block_cached__gqa_block_cached__near_ridge_kernel(
    A_x: jax.Array,
    A_k_cache: jax.Array,
    A_v_cache: jax.Array,
    A_wq: jax.Array,
    A_wo: jax.Array,
    B_x: jax.Array,
    B_k_cache: jax.Array,
    B_v_cache: jax.Array,
    B_wq: jax.Array,
    B_wo: jax.Array,
):
    B, Sq, D = A_x.shape
    _, Hkv, Sk, Dh = A_k_cache.shape
    assert Hkv == HQ and Dh == DH
    n_steps = B * NHP

    kta = jnp.swapaxes(A_k_cache, 2, 3)
    vta = jnp.swapaxes(A_v_cache, 2, 3)
    ktb = jnp.swapaxes(B_k_cache, 2, 3)
    vtb = jnp.swapaxes(B_v_cache, 2, 3)

    def tq(t):
        return jnp.minimum(t, n_steps - 1)

    def tp(t):
        return jnp.maximum(t - 2, 0)

    x_spec = pl.BlockSpec((1, Sq, D), lambda t: (tq(t) // NHP, 0, 0))
    k_spec = pl.BlockSpec((1, HP, Dh, Sk), lambda t: (tq(t) // NHP, tq(t) % NHP, 0, 0))
    v_spec = pl.BlockSpec((1, HP, Dh, Sk), lambda t: (tp(t) // NHP, tp(t) % NHP, 0, 0))
    wq_spec = pl.BlockSpec((D, HQ * DH), lambda t: (0, 0))
    wo_spec = pl.BlockSpec((HQ * DH, D), lambda t: (0, 0))
    in_specs = [x_spec, k_spec, v_spec, wq_spec, wo_spec] * 2

    return pl.pallas_call(
        functools.partial(_attn_kernel, d_model=D, n_steps=n_steps),
        grid=(n_steps + 2,),
        in_specs=in_specs,
        out_specs=pl.BlockSpec((1, Sq, 2 * D), lambda t: (tp(t) // NHP, 0, 0)),
        out_shape=jax.ShapeDtypeStruct((B, Sq, 2 * D), A_x.dtype),
        scratch_shapes=[
            pltpu.VMEM((2 * HP, Sq, Sk), jnp.float32),
            pltpu.VMEM((2 * HP, Sq, Sk), jnp.float32),
            pltpu.VMEM((2 * HP, Sq, Sk), jnp.bfloat16),
            pltpu.VMEM((2 * HP, Sq, Sk), jnp.bfloat16),
            pltpu.VMEM((Sq, D), jnp.float32),
            pltpu.VMEM((Sq, D), jnp.float32),
        ],
        compiler_params=pltpu.CompilerParams(
            dimension_semantics=("arbitrary",),
            vmem_limit_bytes=100 * 1024 * 1024,
        ),
    )(A_x, kta, vta, A_wq, A_wo,
      B_x, ktb, vtb, B_wq, B_wo)
```

```python
import functools

import jax
import jax.numpy as jnp
import jax.experimental.pallas as pl
import jax.experimental.pallas.tpu as pltpu

HQ = 32
DH = 192
HP = 2
NHP = HQ // HP
ROWS = 48


def _attn_kernel(xa_ref, kta_ref, vta_ref, wqa_ref, woa_ref,
                 xb_ref, ktb_ref, vtb_ref, wqb_ref, wob_ref,
                 o_ref, s_ref, p_ref, acca_ref, accb_ref,
                 *, d_model, n_steps):
    t = pl.program_id(0)
    scale = DH ** -0.5
    w = HP * DH
    sq = xa_ref.shape[1]
    hp_q = jnp.minimum(t, n_steps - 1) % NHP
    hp_p = jnp.maximum(t - 2, 0) % NHP

    @pl.when(t == 0)
    def _():
        for r in (s_ref, p_ref):
            r[...] = jnp.zeros(r.shape, r.dtype)

    probs = ((xa_ref, kta_ref, vta_ref, wqa_ref, woa_ref, acca_ref),
             (xb_ref, ktb_ref, vtb_ref, wqb_ref, wob_ref, accb_ref))

    colq = pl.multiple_of(hp_q * w, 128)
    colp = pl.multiple_of(hp_p * w, 128)
    for pi, (x_ref, kt_ref, vt_ref, wq_ref, wo_ref, acc_ref) in enumerate(probs):
        q2 = jnp.dot(x_ref[0], wq_ref[:, pl.ds(colq, w)],
                     preferred_element_type=jnp.float32)
        q2 = (q2 * scale).astype(jnp.bfloat16)
        outs = []
        for j in range(HP):
            i = pi * HP + j
            o = jax.lax.dot_general(p_ref[i], vt_ref[0, j],
                                    (((1,), (1,)), ((), ())),
                                    preferred_element_type=jnp.float32)
            outs.append(o.astype(jnp.bfloat16))
            for r0 in range(0, sq, ROWS):
                s = s_ref[i, r0:r0 + ROWS, :]
                m = jnp.max(s, axis=-1, keepdims=True)
                e = jnp.exp(s - m)
                l = jnp.sum(e, axis=-1, keepdims=True)
                p_ref[i, r0:r0 + ROWS, :] = (e * (1.0 / l)).astype(jnp.bfloat16)
                lmin = jnp.min(l) if r0 == 0 else jnp.minimum(lmin, jnp.min(l))
            z = (lmin < 0.0).astype(jnp.int32)
            q = q2[:, j * DH:(j + 1) * DH]
            s_ref[i] = jnp.dot(q, kt_ref[0, j + z], preferred_element_type=jnp.float32)
        o2 = jnp.concatenate(outs, axis=-1)
        contrib = jnp.dot(o2, wo_ref[pl.ds(colp, w), :],
                          preferred_element_type=jnp.float32)
        acc_ref[...] = jnp.where(hp_p == 0, 0.0, acc_ref[...]) + contrib

    @pl.when(jnp.logical_and(t >= 2, hp_p == NHP - 1))
    def _():
        o_ref[0, :, :d_model] = acca_ref[...].astype(o_ref.dtype)
        o_ref[0, :, d_model:] = accb_ref[...].astype(o_ref.dtype)


@jax.jit
def pallas_concat_heads__gqa_block_cached__gqa_block_cached__near_ridge_kernel(
    A_x: jax.Array,
    A_k_cache: jax.Array,
    A_v_cache: jax.Array,
    A_wq: jax.Array,
    A_wo: jax.Array,
    B_x: jax.Array,
    B_k_cache: jax.Array,
    B_v_cache: jax.Array,
    B_wq: jax.Array,
    B_wo: jax.Array,
):
    B, Sq, D = A_x.shape
    _, Hkv, Sk, Dh = A_k_cache.shape
    assert Hkv == HQ and Dh == DH
    n_steps = B * NHP

    kta = jnp.swapaxes(A_k_cache, 2, 3)
    vta = jnp.swapaxes(A_v_cache, 2, 3)
    ktb = jnp.swapaxes(B_k_cache, 2, 3)
    vtb = jnp.swapaxes(B_v_cache, 2, 3)

    def tq(t):
        return jnp.minimum(t, n_steps - 1)

    def tp(t):
        return jnp.maximum(t - 2, 0)

    x_spec = pl.BlockSpec((1, Sq, D), lambda t: (tq(t) // NHP, 0, 0))
    k_spec = pl.BlockSpec((1, HP, Dh, Sk), lambda t: (tq(t) // NHP, tq(t) % NHP, 0, 0))
    v_spec = pl.BlockSpec((1, HP, Dh, Sk), lambda t: (tp(t) // NHP, tp(t) % NHP, 0, 0))
    wq_spec = pl.BlockSpec((D, HQ * DH), lambda t: (0, 0))
    wo_spec = pl.BlockSpec((HQ * DH, D), lambda t: (0, 0))
    in_specs = [x_spec, k_spec, v_spec, wq_spec, wo_spec] * 2

    return pl.pallas_call(
        functools.partial(_attn_kernel, d_model=D, n_steps=n_steps),
        grid=(n_steps + 2,),
        in_specs=in_specs,
        out_specs=pl.BlockSpec((1, Sq, 2 * D), lambda t: (tp(t) // NHP, 0, 0)),
        out_shape=jax.ShapeDtypeStruct((B, Sq, 2 * D), A_x.dtype),
        scratch_shapes=[
            pltpu.VMEM((2 * HP, Sq, Sk), jnp.float32),
            pltpu.VMEM((2 * HP, Sq, Sk), jnp.bfloat16),
            pltpu.VMEM((Sq, D), jnp.float32),
            pltpu.VMEM((Sq, D), jnp.float32),
        ],
        compiler_params=pltpu.CompilerParams(
            dimension_semantics=("arbitrary",),
            vmem_limit_bytes=100 * 1024 * 1024,
        ),
    )(A_x, kta, vta, A_wq, A_wo,
      B_x, ktb, vtb, B_wq, B_wo)
```

```python
import functools

import jax
import jax.numpy as jnp
import jax.experimental.pallas as pl
import jax.experimental.pallas.tpu as pltpu

HQ = 32
DH = 192
HP = 2
NHP = HQ // HP
ROWS = 48


def _attn_kernel(xa_ref, kta_ref, vta_ref, wqa_ref, woa_ref,
                 xb_ref, ktb_ref, vtb_ref, wqb_ref, wob_ref,
                 o_ref, s_ref, p_ref, acca_ref, accb_ref,
                 *, d_model, n_steps):
    t = pl.program_id(0)
    scale = DH ** -0.5
    w = HP * DH
    sq = xa_ref.shape[1]
    hp_q = jnp.minimum(t, n_steps - 1) % NHP
    hp_p = jnp.maximum(t - 2, 0) % NHP

    @pl.when(t == 0)
    def _():
        for r in (s_ref, p_ref):
            r[...] = jnp.zeros(r.shape, r.dtype)

    probs = ((xa_ref, kta_ref, vta_ref, wqa_ref, woa_ref, acca_ref),
             (xb_ref, ktb_ref, vtb_ref, wqb_ref, wob_ref, accb_ref))

    colq = pl.multiple_of(hp_q * w, 128)
    colp = pl.multiple_of(hp_p * w, 128)
    q2s = []
    for x_ref, _, _, wq_ref, _, _ in probs:
        q2 = jnp.dot(x_ref[0], wq_ref[:, pl.ds(colq, w)],
                     preferred_element_type=jnp.float32)
        q2s.append((q2 * scale).astype(jnp.bfloat16))
    for pi, (x_ref, kt_ref, vt_ref, wq_ref, wo_ref, acc_ref) in enumerate(probs):
        q2 = q2s[pi]
        outs = []
        for j in range(HP):
            i = pi * HP + j
            o = jax.lax.dot_general(p_ref[i], vt_ref[0, j],
                                    (((1,), (1,)), ((), ())),
                                    preferred_element_type=jnp.float32)
            outs.append(o.astype(jnp.bfloat16))
            for r0 in range(0, sq, ROWS):
                s = s_ref[i, r0:r0 + ROWS, :]
                m = jnp.max(s, axis=-1, keepdims=True)
                e = jnp.exp(s - m)
                l = jnp.sum(e, axis=-1, keepdims=True)
                p_ref[i, r0:r0 + ROWS, :] = (e * (1.0 / l)).astype(jnp.bfloat16)
                lmin = jnp.min(l) if r0 == 0 else jnp.minimum(lmin, jnp.min(l))
            z = (lmin < 0.0).astype(jnp.int32)
            q = q2[:, j * DH:(j + 1) * DH]
            s_ref[i] = jnp.dot(q, kt_ref[0, j + z], preferred_element_type=jnp.float32)
        o2 = jnp.concatenate(outs, axis=-1)
        contrib = jnp.dot(o2, wo_ref[pl.ds(colp, w), :],
                          preferred_element_type=jnp.float32)
        acc_ref[...] = jnp.where(hp_p == 0, 0.0, acc_ref[...]) + contrib

    @pl.when(jnp.logical_and(t >= 2, hp_p == NHP - 1))
    def _():
        o_ref[0, :, :d_model] = acca_ref[...].astype(o_ref.dtype)
        o_ref[0, :, d_model:] = accb_ref[...].astype(o_ref.dtype)


@jax.jit
def pallas_concat_heads__gqa_block_cached__gqa_block_cached__near_ridge_kernel(
    A_x: jax.Array,
    A_k_cache: jax.Array,
    A_v_cache: jax.Array,
    A_wq: jax.Array,
    A_wo: jax.Array,
    B_x: jax.Array,
    B_k_cache: jax.Array,
    B_v_cache: jax.Array,
    B_wq: jax.Array,
    B_wo: jax.Array,
):
    B, Sq, D = A_x.shape
    _, Hkv, Sk, Dh = A_k_cache.shape
    assert Hkv == HQ and Dh == DH
    n_steps = B * NHP

    kta = jnp.swapaxes(A_k_cache, 2, 3)
    vta = jnp.swapaxes(A_v_cache, 2, 3)
    ktb = jnp.swapaxes(B_k_cache, 2, 3)
    vtb = jnp.swapaxes(B_v_cache, 2, 3)

    def tq(t):
        return jnp.minimum(t, n_steps - 1)

    def tp(t):
        return jnp.maximum(t - 2, 0)

    x_spec = pl.BlockSpec((1, Sq, D), lambda t: (tq(t) // NHP, 0, 0))
    k_spec = pl.BlockSpec((1, HP, Dh, Sk), lambda t: (tq(t) // NHP, tq(t) % NHP, 0, 0))
    v_spec = pl.BlockSpec((1, HP, Dh, Sk), lambda t: (tp(t) // NHP, tp(t) % NHP, 0, 0))
    wq_spec = pl.BlockSpec((D, HQ * DH), lambda t: (0, 0))
    wo_spec = pl.BlockSpec((HQ * DH, D), lambda t: (0, 0))
    in_specs = [x_spec, k_spec, v_spec, wq_spec, wo_spec] * 2

    return pl.pallas_call(
        functools.partial(_attn_kernel, d_model=D, n_steps=n_steps),
        grid=(n_steps + 2,),
        in_specs=in_specs,
        out_specs=pl.BlockSpec((1, Sq, 2 * D), lambda t: (tp(t) // NHP, 0, 0)),
        out_shape=jax.ShapeDtypeStruct((B, Sq, 2 * D), A_x.dtype),
        scratch_shapes=[
            pltpu.VMEM((2 * HP, Sq, Sk), jnp.float32),
            pltpu.VMEM((2 * HP, Sq, Sk), jnp.bfloat16),
            pltpu.VMEM((Sq, D), jnp.float32),
            pltpu.VMEM((Sq, D), jnp.float32),
        ],
        compiler_params=pltpu.CompilerParams(
            dimension_semantics=("arbitrary",),
            vmem_limit_bytes=100 * 1024 * 1024,
        ),
    )(A_x, kta, vta, A_wq, A_wo,
      B_x, ktb, vtb, B_wq, B_wo)
```

```python
import functools

import jax
import jax.numpy as jnp
import jax.experimental.pallas as pl
import jax.experimental.pallas.tpu as pltpu

HQ = 32
DH = 192
HP = 2
NHP = HQ // HP
ROWS = 48
LOG2E = 1.4426950408889634


def _attn_kernel(xa_ref, kta_ref, vta_ref, wqa_ref, woa_ref,
                 xb_ref, ktb_ref, vtb_ref, wqb_ref, wob_ref,
                 o_ref, s_ref, p_ref, l_ref, acca_ref, accb_ref,
                 *, d_model, n_steps):
    t = pl.program_id(0)
    scale = DH ** -0.5 * LOG2E
    w = HP * DH
    sq = xa_ref.shape[1]
    hp_q = jnp.minimum(t, n_steps - 1) % NHP
    hp_p = jnp.maximum(t - 2, 0) % NHP

    @pl.when(t == 0)
    def _():
        for r in (s_ref, p_ref, l_ref):
            r[...] = jnp.zeros(r.shape, r.dtype)

    probs = ((xa_ref, kta_ref, vta_ref, wqa_ref, woa_ref, acca_ref),
             (xb_ref, ktb_ref, vtb_ref, wqb_ref, wob_ref, accb_ref))

    colq = pl.multiple_of(hp_q * w, 128)
    colp = pl.multiple_of(hp_p * w, 128)
    for pi, (x_ref, kt_ref, vt_ref, wq_ref, wo_ref, acc_ref) in enumerate(probs):
        q2 = jnp.dot(x_ref[0], wq_ref[:, pl.ds(colq, w)],
                     preferred_element_type=jnp.float32)
        q2 = (q2 * scale).astype(jnp.bfloat16)
        outs = []
        for j in range(HP):
            i = pi * HP + j
            o = jax.lax.dot_general(vt_ref[0, j], p_ref[i],
                                    (((1,), (1,)), ((), ())),
                                    preferred_element_type=jnp.float32).T
            outs.append((o / l_ref[i]).astype(jnp.bfloat16))
            for r0 in range(0, sq, ROWS):
                s = s_ref[i, r0:r0 + ROWS, :]
                m = jnp.max(s, axis=-1, keepdims=True)
                e = jnp.exp2(s - m)
                l = jnp.sum(e, axis=-1, keepdims=True)
                p_ref[i, r0:r0 + ROWS, :] = e.astype(jnp.bfloat16)
                l_ref[i, r0:r0 + ROWS, :] = l
                lmin = jnp.min(l) if r0 == 0 else jnp.minimum(lmin, jnp.min(l))
            z = (lmin < 0.0).astype(jnp.int32)
            q = q2[:, j * DH:(j + 1) * DH]
            s_ref[i] = jnp.dot(q, kt_ref[0, j + z], preferred_element_type=jnp.float32)
        o2 = jnp.concatenate(outs, axis=-1)
        contrib = jnp.dot(o2, wo_ref[pl.ds(colp, w), :],
                          preferred_element_type=jnp.float32)
        acc_ref[...] = jnp.where(hp_p == 0, 0.0, acc_ref[...]) + contrib

    @pl.when(jnp.logical_and(t >= 2, hp_p == NHP - 1))
    def _():
        o_ref[0, :, :d_model] = acca_ref[...].astype(o_ref.dtype)
        o_ref[0, :, d_model:] = accb_ref[...].astype(o_ref.dtype)


@jax.jit
def pallas_concat_heads__gqa_block_cached__gqa_block_cached__near_ridge_kernel(
    A_x: jax.Array,
    A_k_cache: jax.Array,
    A_v_cache: jax.Array,
    A_wq: jax.Array,
    A_wo: jax.Array,
    B_x: jax.Array,
    B_k_cache: jax.Array,
    B_v_cache: jax.Array,
    B_wq: jax.Array,
    B_wo: jax.Array,
):
    B, Sq, D = A_x.shape
    _, Hkv, Sk, Dh = A_k_cache.shape
    assert Hkv == HQ and Dh == DH
    n_steps = B * NHP

    kta = jnp.swapaxes(A_k_cache, 2, 3)
    vta = jnp.swapaxes(A_v_cache, 2, 3)
    ktb = jnp.swapaxes(B_k_cache, 2, 3)
    vtb = jnp.swapaxes(B_v_cache, 2, 3)

    def tq(t):
        return jnp.minimum(t, n_steps - 1)

    def tp(t):
        return jnp.maximum(t - 2, 0)

    x_spec = pl.BlockSpec((1, Sq, D), lambda t: (tq(t) // NHP, 0, 0))
    k_spec = pl.BlockSpec((1, HP, Dh, Sk), lambda t: (tq(t) // NHP, tq(t) % NHP, 0, 0))
    v_spec = pl.BlockSpec((1, HP, Dh, Sk), lambda t: (tp(t) // NHP, tp(t) % NHP, 0, 0))
    wq_spec = pl.BlockSpec((D, HQ * DH), lambda t: (0, 0))
    wo_spec = pl.BlockSpec((HQ * DH, D), lambda t: (0, 0))
    in_specs = [x_spec, k_spec, v_spec, wq_spec, wo_spec] * 2

    return pl.pallas_call(
        functools.partial(_attn_kernel, d_model=D, n_steps=n_steps),
        grid=(n_steps + 2,),
        in_specs=in_specs,
        out_specs=pl.BlockSpec((1, Sq, 2 * D), lambda t: (tp(t) // NHP, 0, 0)),
        out_shape=jax.ShapeDtypeStruct((B, Sq, 2 * D), A_x.dtype),
        scratch_shapes=[
            pltpu.VMEM((2 * HP, Sq, Sk), jnp.float32),
            pltpu.VMEM((2 * HP, Sq, Sk), jnp.bfloat16),
            pltpu.VMEM((2 * HP, Sq, 1), jnp.float32),
            pltpu.VMEM((Sq, D), jnp.float32),
            pltpu.VMEM((Sq, D), jnp.float32),
        ],
        compiler_params=pltpu.CompilerParams(
            dimension_semantics=("arbitrary",),
            vmem_limit_bytes=100 * 1024 * 1024,
        ),
    )(A_x, kta, vta, A_wq, A_wo,
      B_x, ktb, vtb, B_wq, B_wo)
```

```python
import functools

import jax
import jax.numpy as jnp
import jax.experimental.pallas as pl
import jax.experimental.pallas.tpu as pltpu

HQ = 32
DH = 192
HP = 2
NHP = HQ // HP
ROWS = 48
LOG2E = 1.4426950408889634


def _attn_kernel(xa_ref, kta_ref, vta_ref, wqa_ref, woa_ref,
                 xb_ref, ktb_ref, vtb_ref, wqb_ref, wob_ref,
                 o_ref, s_ref, p_ref, l_ref, acca_ref, accb_ref,
                 *, d_model, n_steps):
    t = pl.program_id(0)
    scale = DH ** -0.5 * LOG2E
    w = HP * DH
    sq = xa_ref.shape[1]
    hp_q = jnp.minimum(t, n_steps - 1) % NHP
    hp_p = jnp.maximum(t - 2, 0) % NHP

    @pl.when(t == 0)
    def _():
        for r in (s_ref, p_ref, l_ref):
            r[...] = jnp.zeros(r.shape, r.dtype)

    probs = ((xa_ref, kta_ref, vta_ref, wqa_ref, woa_ref, acca_ref),
             (xb_ref, ktb_ref, vtb_ref, wqb_ref, wob_ref, accb_ref))

    colq = pl.multiple_of(hp_q * w, 128)
    colp = pl.multiple_of(hp_p * w, 128)
    zs = []
    for pi, (x_ref, kt_ref, vt_ref, wq_ref, wo_ref, acc_ref) in enumerate(probs):
        q2 = jnp.dot(x_ref[0], wq_ref[:, pl.ds(colq, w)],
                     preferred_element_type=jnp.float32)
        q2 = (q2 * scale).astype(jnp.bfloat16)
        outs = []
        for j in range(HP):
            i = pi * HP + j
            zp = zs[i - 2] if i >= 2 else 0
            o = jax.lax.dot_general(vt_ref[0, j + zp], p_ref[i],
                                    (((1,), (1,)), ((), ())),
                                    preferred_element_type=jnp.float32).T
            outs.append((o / l_ref[i]).astype(jnp.bfloat16))
            for r0 in range(0, sq, ROWS):
                s = s_ref[i, r0:r0 + ROWS, :]
                m = jnp.max(s, axis=-1, keepdims=True)
                e = jnp.exp2(s - m)
                l = jnp.sum(e, axis=-1, keepdims=True)
                p_ref[i, r0:r0 + ROWS, :] = e.astype(jnp.bfloat16)
                l_ref[i, r0:r0 + ROWS, :] = l
                lmin = jnp.min(l) if r0 == 0 else jnp.minimum(lmin, jnp.min(l))
            z = (lmin < 0.0).astype(jnp.int32)
            zs.append(z)
            q = q2[:, j * DH:(j + 1) * DH]
            s_ref[i] = jnp.dot(q, kt_ref[0, j + z], preferred_element_type=jnp.float32)
        o2 = jnp.concatenate(outs, axis=-1)
        contrib = jnp.dot(o2, wo_ref[pl.ds(colp, w), :],
                          preferred_element_type=jnp.float32)
        acc_ref[...] = jnp.where(hp_p == 0, 0.0, acc_ref[...]) + contrib

    @pl.when(jnp.logical_and(t >= 2, hp_p == NHP - 1))
    def _():
        o_ref[0, :, :d_model] = acca_ref[...].astype(o_ref.dtype)
        o_ref[0, :, d_model:] = accb_ref[...].astype(o_ref.dtype)


@jax.jit
def pallas_concat_heads__gqa_block_cached__gqa_block_cached__near_ridge_kernel(
    A_x: jax.Array,
    A_k_cache: jax.Array,
    A_v_cache: jax.Array,
    A_wq: jax.Array,
    A_wo: jax.Array,
    B_x: jax.Array,
    B_k_cache: jax.Array,
    B_v_cache: jax.Array,
    B_wq: jax.Array,
    B_wo: jax.Array,
):
    B, Sq, D = A_x.shape
    _, Hkv, Sk, Dh = A_k_cache.shape
    assert Hkv == HQ and Dh == DH
    n_steps = B * NHP

    kta = jnp.swapaxes(A_k_cache, 2, 3)
    vta = jnp.swapaxes(A_v_cache, 2, 3)
    ktb = jnp.swapaxes(B_k_cache, 2, 3)
    vtb = jnp.swapaxes(B_v_cache, 2, 3)

    def tq(t):
        return jnp.minimum(t, n_steps - 1)

    def tp(t):
        return jnp.maximum(t - 2, 0)

    x_spec = pl.BlockSpec((1, Sq, D), lambda t: (tq(t) // NHP, 0, 0))
    k_spec = pl.BlockSpec((1, HP, Dh, Sk), lambda t: (tq(t) // NHP, tq(t) % NHP, 0, 0))
    v_spec = pl.BlockSpec((1, HP, Dh, Sk), lambda t: (tp(t) // NHP, tp(t) % NHP, 0, 0))
    wq_spec = pl.BlockSpec((D, HQ * DH), lambda t: (0, 0))
    wo_spec = pl.BlockSpec((HQ * DH, D), lambda t: (0, 0))
    in_specs = [x_spec, k_spec, v_spec, wq_spec, wo_spec] * 2

    return pl.pallas_call(
        functools.partial(_attn_kernel, d_model=D, n_steps=n_steps),
        grid=(n_steps + 2,),
        in_specs=in_specs,
        out_specs=pl.BlockSpec((1, Sq, 2 * D), lambda t: (tp(t) // NHP, 0, 0)),
        out_shape=jax.ShapeDtypeStruct((B, Sq, 2 * D), A_x.dtype),
        scratch_shapes=[
            pltpu.VMEM((2 * HP, Sq, Sk), jnp.float32),
            pltpu.VMEM((2 * HP, Sq, Sk), jnp.bfloat16),
            pltpu.VMEM((2 * HP, Sq, 1), jnp.float32),
            pltpu.VMEM((Sq, D), jnp.float32),
            pltpu.VMEM((Sq, D), jnp.float32),
        ],
        compiler_params=pltpu.CompilerParams(
            dimension_semantics=("arbitrary",),
            vmem_limit_bytes=100 * 1024 * 1024,
        ),
    )(A_x, kta, vta, A_wq, A_wo,
      B_x, ktb, vtb, B_wq, B_wo)
```

```python
import functools

import jax
import jax.numpy as jnp
import jax.experimental.pallas as pl
import jax.experimental.pallas.tpu as pltpu

HQ = 32
DH = 192
HP = 2
NHP = HQ // HP
ROWS = 48
LOG2E = 1.4426950408889634
ORDER = "P2 P0 S0 P3 X0 X1 S2 P1 S1 Q2 O0 Q1 O1 S3 Q0 Q3"


def _attn_kernel(xa_ref, kta_ref, vta_ref, wqa_hbm, woa_hbm,
                 xb_ref, ktb_ref, vtb_ref, wqb_hbm, wob_hbm,
                 o_ref, s_ref, p_ref, l_ref, acca_ref, accb_ref,
                 wqa_ref, woa_ref, wqb_ref, wob_ref, sems,
                 *, d_model, n_steps):
    t = pl.program_id(0)
    scale = DH ** -0.5 * LOG2E
    w = HP * DH
    sq = xa_ref.shape[1]
    hp_q = jnp.minimum(t, n_steps - 1) % NHP
    hp_p = jnp.maximum(t - 2, 0) % NHP

    def wq_copy(pi, g):
        src, dst = ((wqa_hbm, wqa_ref), (wqb_hbm, wqb_ref))[pi]
        cols = pl.ds(pl.multiple_of(g * w, 128), w)
        return pltpu.make_async_copy(src.at[:, cols], dst.at[:, cols], sems.at[pi, g])

    def wo_copy(pi, g):
        src, dst = ((woa_hbm, woa_ref), (wob_hbm, wob_ref))[pi]
        rows = pl.ds(pl.multiple_of(g * w, 128), w)
        return pltpu.make_async_copy(src.at[rows, :], dst.at[rows, :], sems.at[2 + pi, g])

    def start_copies(g):
        for pi in range(2):
            wq_copy(pi, g).start()
        for pi in range(2):
            wo_copy(pi, g).start()

    @pl.when(t == 0)
    def _():
        start_copies(0)
        start_copies(1)

    @pl.when(t + 2 < NHP)
    def _():
        start_copies(t + 2)

    @pl.when(t < NHP)
    def _():
        for pi in range(2):
            wq_copy(pi, t).wait()
            wo_copy(pi, t).wait()

    probs = ((xa_ref, kta_ref, vta_ref, wqa_ref, woa_ref, acca_ref),
             (xb_ref, ktb_ref, vtb_ref, wqb_ref, wob_ref, accb_ref))
    colq = pl.multiple_of(hp_q * w, 128)
    colp = pl.multiple_of(hp_p * w, 128)

    def run(kinds):
        z = [0] * (2 * HP)
        outs = [None] * (2 * HP)
        q2 = [None, None]

        def qproj(pi):
            x_ref, _, _, wq_ref, _, _ = probs[pi]
            r = jnp.dot(x_ref[0], wq_ref[:, pl.ds(colq, w)],
                        preferred_element_type=jnp.float32)
            q2[pi] = (r * scale).astype(jnp.bfloat16)

        def pv(i):
            pi, j = divmod(i, HP)
            o = jax.lax.dot_general(probs[pi][2][0, j], p_ref[i],
                                    (((1,), (1,)), ((), ())),
                                    preferred_element_type=jnp.float32).T
            outs[i] = (o / l_ref[i]).astype(jnp.bfloat16)

        def softmax(i):
            lmin = None
            for r0 in range(0, sq, ROWS):
                s = s_ref[i, r0:r0 + ROWS, :]
                m = jnp.max(s, axis=-1, keepdims=True)
                e = jnp.exp2(s - m)
                l = jnp.sum(e, axis=-1, keepdims=True)
                p_ref[i, r0:r0 + ROWS, :] = e.astype(jnp.bfloat16)
                l_ref[i, r0:r0 + ROWS, :] = l
                lmin = jnp.min(l) if lmin is None else jnp.minimum(lmin, jnp.min(l))
            z[i] = (lmin < 0.0).astype(jnp.int32)

        def qk(i):
            pi, j = divmod(i, HP)
            q = q2[pi][:, j * DH:(j + 1) * DH]
            s_ref[i] = jnp.dot(q, probs[pi][1][0, j + z[i]],
                               preferred_element_type=jnp.float32)

        def oproj(pi):
            wo_ref, acc_ref = probs[pi][4], probs[pi][5]
            o2 = jnp.concatenate(outs[pi * HP:(pi + 1) * HP], axis=-1)
            contrib = jnp.dot(o2, wo_ref[pl.ds(colp, w), :],
                              preferred_element_type=jnp.float32)
            acc_ref[...] = jnp.where(hp_p == 0, 0.0, acc_ref[...]) + contrib

        stages = dict(P=pv, S=softmax, Q=qk, X=qproj, O=oproj)
        for op in ORDER.split():
            if op[0] in kinds:
                stages[op[0]](int(op[1]))

    pl.when(t == 0)(lambda: run("XQ"))
    pl.when(t == 1)(lambda: run("SXQ"))
    pl.when(jnp.logical_and(t >= 2, t < n_steps))(lambda: run("PSXQO"))
    pl.when(t == n_steps)(lambda: run("POS"))
    pl.when(t == n_steps + 1)(lambda: run("PO"))

    @pl.when(jnp.logical_and(t >= 2, hp_p == NHP - 1))
    def _():
        o_ref[0, :, :d_model] = acca_ref[...].astype(o_ref.dtype)
        o_ref[0, :, d_model:] = accb_ref[...].astype(o_ref.dtype)


@jax.jit
def pallas_concat_heads__gqa_block_cached__gqa_block_cached__near_ridge_kernel(
    A_x: jax.Array,
    A_k_cache: jax.Array,
    A_v_cache: jax.Array,
    A_wq: jax.Array,
    A_wo: jax.Array,
    B_x: jax.Array,
    B_k_cache: jax.Array,
    B_v_cache: jax.Array,
    B_wq: jax.Array,
    B_wo: jax.Array,
):
    B, Sq, D = A_x.shape
    _, Hkv, Sk, Dh = A_k_cache.shape
    assert Hkv == HQ and Dh == DH
    n_steps = B * NHP

    kta = jnp.swapaxes(A_k_cache, 2, 3)
    vta = jnp.swapaxes(A_v_cache, 2, 3)
    ktb = jnp.swapaxes(B_k_cache, 2, 3)
    vtb = jnp.swapaxes(B_v_cache, 2, 3)

    def item(t, lag):
        return jnp.clip(t - lag, 0, n_steps - 1)

    x_spec = pl.BlockSpec((1, Sq, D), lambda t: (item(t, 0) // NHP, 0, 0))
    k_spec = pl.BlockSpec((1, HP, Dh, Sk),
                          lambda t: (item(t, 0) // NHP, item(t, 0) % NHP, 0, 0))
    v_spec = pl.BlockSpec((1, HP, Dh, Sk),
                          lambda t: (item(t, 2) // NHP, item(t, 2) % NHP, 0, 0))
    w_spec = pl.BlockSpec(memory_space=pl.ANY)
    in_specs = [x_spec, k_spec, v_spec, w_spec, w_spec] * 2

    return pl.pallas_call(
        functools.partial(_attn_kernel, d_model=D, n_steps=n_steps),
        grid=(n_steps + 2,),
        in_specs=in_specs,
        out_specs=pl.BlockSpec((1, Sq, 2 * D), lambda t: (item(t, 2) // NHP, 0, 0)),
        out_shape=jax.ShapeDtypeStruct((B, Sq, 2 * D), A_x.dtype),
        scratch_shapes=[
            pltpu.VMEM((2 * HP, Sq, Sk), jnp.float32),
            pltpu.VMEM((2 * HP, Sq, Sk), jnp.bfloat16),
            pltpu.VMEM((2 * HP, Sq, 1), jnp.float32),
            pltpu.VMEM((Sq, D), jnp.float32),
            pltpu.VMEM((Sq, D), jnp.float32),
            pltpu.VMEM((D, HQ * DH), A_wq.dtype),
            pltpu.VMEM((HQ * DH, D), A_wo.dtype),
            pltpu.VMEM((D, HQ * DH), B_wq.dtype),
            pltpu.VMEM((HQ * DH, D), B_wo.dtype),
            pltpu.SemaphoreType.DMA((4, NHP)),
        ],
        compiler_params=pltpu.CompilerParams(
            dimension_semantics=("arbitrary",),
            vmem_limit_bytes=100 * 1024 * 1024,
        ),
    )(A_x, kta, vta, A_wq, A_wo,
      B_x, ktb, vtb, B_wq, B_wo)
```
